```python
import jax
import jax.numpy as jnp

def _softmax(x, axis=-1):
    return jax.nn.softmax(x, axis=axis)

def _gelu(x):
    return jax.nn.gelu(x, approximate=True)

def _silu(x):
    return jax.nn.silu(x)

def _sigmoid(x):
    return jax.nn.sigmoid(x)

def _layernorm(x, axis=-1, eps=1e-05):
    m = jnp.mean(x, axis=axis, keepdims=True)
    v = jnp.var(x, axis=axis, keepdims=True)
    return (x - m) / jnp.sqrt(v + eps)

def _scatter_add(tgt, idx, src, axis=0):
    return tgt.at[idx].add(src)

def _segment_sum(src, seg, n):
    return jax.ops.segment_sum(src, seg, n)

class _Rng:

    def __init__(self, key):
        self._k = key

    def _next(self):
        self._k, sub = jax.random.split(self._k)
        return sub

    def normal(self, shape):
        return jax.random.normal(self._next(), shape, dtype=jnp.bfloat16)

    def randint(self, lo, hi, shape):
        return jax.random.randint(self._next(), shape, lo, hi, dtype=jnp.int32)

    def uniform(self, shape, lo=0.0, hi=1.0):
        return jax.random.uniform(self._next(), shape, jnp.bfloat16, lo, hi)

    def permutation(self, n):
        return jax.random.permutation(self._next(), n)
kernel_name = 'adaLN_cond__sliding_block_cached__glu_gated_swiglu__decode'

def setup_inputs():
    _rng = _Rng(jax.random.key(int.from_bytes(__import__("os").urandom(4), "little")))
    _w = lambda a: (lambda t: t.astype(jnp.bfloat16) if jnp.issubdtype(t.dtype, jnp.floating) else t)(jnp.asarray(a))

    def _A_setup():
        B, Sq, D = (2, 1, 512)
        Hq, Hkv, Sk, Dh = (32, 32, 16384, 128)
        assert Hq % Hkv == 0, (Hq, Hkv)
        return {'x': _w((lambda *s: _rng.normal(s) * 0.05)(B, Sq, D)), 'k_cache': _w((lambda *s: _rng.normal(s) * 0.05)(B, Hkv, Sk, Dh)), 'v_cache': _w((lambda *s: _rng.normal(s) * 0.05)(B, Hkv, Sk, Dh)), 'wq': _w((lambda *s: _rng.normal(s) * 0.05)(D, Hq * Dh) * D ** (-0.5)), 'wo': _w((lambda *s: _rng.normal(s) * 0.05)(Hq * Dh, D) * (Hq * Dh) ** (-0.5))}
    _A_in = _A_setup()

    def _B_setup():
        B, S, D, F = (2, 1, 512, 1376)
        return {'x': _w((lambda *s: _rng.normal(s) * 0.05)(B, S, D)), 'w1': _w((lambda *s: _rng.normal(s) * 0.05)(D, F) * (2.0 / D) ** 0.5), 'w3': _w((lambda *s: _rng.normal(s) * 0.05)(D, F) * (2.0 / D) ** 0.5), 'w2': _w((lambda *s: _rng.normal(s) * 0.05)(F, D) * (2.0 / F) ** 0.5)}
    _B_in = _B_setup()
    return {'A_x': _A_in['x'], 'A_k_cache': _A_in['k_cache'], 'A_v_cache': _A_in['v_cache'], 'A_wq': _A_in['wq'], 'A_wo': _A_in['wo'], 'B_x': _B_in['x'], 'B_w1': _B_in['w1'], 'B_w3': _B_in['w3'], 'B_w2': _B_in['w2'], 'c': _w((lambda *s: _rng.normal(s) * 0.05)(2, 512)), 'w_mod': _w((lambda *s: _rng.normal(s) * 0.05)(512, 6 * 512) * 512 ** (-0.5))}

def reference(A_x, A_k_cache, A_v_cache, A_wq, A_wo, B_x, B_w1, B_w3, B_w2, c, w_mod):

    def _A_ref(x, k_cache, v_cache, wq, wo):
        B, Sq, D = x.shape
        Hq, Dh = (32, 128)
        Hkv, Sk = (k_cache.shape[1], k_cache.shape[2])
        W = min(4096, max(256, Sk // 4))
        rep = Hq // Hkv
        q = (lambda x, *d: x.transpose(*d))((x @ wq).reshape(B, Sq, Hq, Dh), 0, 2, 1, 3)
        k = jnp.repeat(k_cache[:, :, Sk - W:, :], rep, axis=1)
        v = jnp.repeat(v_cache[:, :, Sk - W:, :], rep, axis=1)
        scores = jnp.einsum('bhqd,bhkd->bhqk', q, k) * Dh ** (-0.5)
        p = _softmax(scores, axis=-1)
        o = jnp.einsum('bhqk,bhkd->bhqd', p, v)
        return (lambda x, *d: x.transpose(*d))(o, 0, 2, 1, 3).reshape(B, Sq, Hq * Dh) @ wo

    def _B_ref(x, w1, w3, w2):
        gate = jnp.einsum('bsd,df->bsf', x, w1)
        up = jnp.einsum('bsd,df->bsf', x, w3)
        h = _silu(gate) * up
        out = jnp.einsum('bsf,fd->bsd', h, w2)
        return out
    x = A_x
    mod = (_silu(c) @ w_mod).reshape(c.shape[0], 6, 1, -1)
    sa, ca, ga, sb, cb, gb = (mod[:, 0].copy(), mod[:, 1].copy(), mod[:, 2].copy(), mod[:, 3].copy(), mod[:, 4].copy(), mod[:, 5].copy())
    h = _layernorm(x, axis=-1) * (1 + ca) + sa
    x = x + ga * _A_ref(h, A_k_cache, A_v_cache, A_wq, A_wo)
    h = _layernorm(x, axis=-1) * (1 + cb) + sb
    x = x + gb * _B_ref(h, B_w1, B_w3, B_w2)
    return x
```

```python
import functools

import jax
import jax.numpy as jnp
import jax.experimental.pallas as pl
import jax.experimental.pallas.tpu as pltpu

F32 = jnp.float32
BF16 = jnp.bfloat16
_NT = (((1,), (1,)), ((), ()))


def _silu(x):
    return x * (1.0 / (1.0 + jnp.exp(-x)))


def _layernorm(x, eps=1e-5):
    m = jnp.mean(x, axis=-1, keepdims=True)
    d = x - m
    v = jnp.mean(d * d, axis=-1, keepdims=True)
    return d / jnp.sqrt(v + eps)


def make(rows=128, ring=3):
    def kern(x_hbm, k_hbm, v_hbm, wq_hbm, wo_hbm, w1_hbm, w3_hbm, w2_hbm, c_hbm, wm_hbm,
             out_hbm,
             x_v, c_v, wm_v, wq_v, wo_v, w1_v, w3_v, w2_v, kv_v, q_v, out_v,
             kv_sem, w_sem):
        B, H, SK, DH = k_hbm.shape
        D = x_hbm.shape[1]
        W = min(4096, max(256, SK // 4))
        nrc = W // rows
        scale = DH ** -0.5

        def kv_start(g, slot):
            for rc in range(nrc):
                for kv, src in enumerate((k_hbm, v_hbm)):
                    for b in range(B):
                        pltpu.make_async_copy(
                            src.at[b, g, pl.ds(SK - W + rc * rows, rows), :],
                            kv_v.at[slot, kv, b, pl.ds(rc * rows, rows), :],
                            kv_sem.at[slot]).start(priority=b % 2)

        def kv_wait(slot):
            pltpu.make_async_copy(kv_v.at[slot], kv_v.at[slot], kv_sem.at[slot]).wait()

        def split_copy(src, dst, sem, n):
            r = src.shape[0] // n
            for i in range(n):
                pltpu.make_async_copy(src.at[pl.ds(i * r, r), :], dst.at[pl.ds(i * r, r), :], sem).start(priority=i % 2)

        def wait_all(dst, sem):
            pltpu.make_async_copy(dst, dst, sem).wait()

        pltpu.make_async_copy(c_hbm, c_v, w_sem.at[0]).start()
        pltpu.make_async_copy(x_hbm, x_v, w_sem.at[1]).start(priority=1)
        split_copy(wm_hbm, wm_v, w_sem.at[2], 16)
        split_copy(wq_hbm, wq_v, w_sem.at[3], 32)
        for g in range(ring - 1):
            kv_start(g, g)
        split_copy(wo_hbm, wo_v, w_sem.at[4], 64)

        wait_all(c_v, w_sem.at[0])
        wait_all(x_v, w_sem.at[1])
        wait_all(wm_v, w_sem.at[2])
        sc = _silu(c_v[...].astype(F32)).astype(BF16)
        mod = jnp.dot(sc, wm_v[...], preferred_element_type=F32)
        x = x_v[...].astype(F32)
        h = _layernorm(x) * (1.0 + mod[:, D:2 * D]) + mod[:, 0:D]
        wait_all(wq_v, w_sem.at[3])
        q = jnp.dot(h.astype(BF16), wq_v[...], preferred_element_type=F32)
        for g in range(H):
            for b in range(B):
                q_v[g, b] = jnp.broadcast_to(q[b:b + 1, g * DH:(g + 1) * DH], (8, DH))

        def head(g, slot, acc):
            outs = []
            for b in range(B):
                qb = q_v[g, b].astype(BF16)
                s = jax.lax.dot_general(qb, kv_v[slot, 0, b], _NT, preferred_element_type=F32)
                m = jnp.max(s, axis=-1, keepdims=True)
                p = jnp.exp((s - m) * scale)
                l = jnp.sum(p, axis=-1, keepdims=True)
                o = jnp.dot(p.astype(BF16), kv_v[slot, 1, b], preferred_element_type=F32)
                outs.append(o / l)
            row = jax.lax.broadcasted_iota(jnp.int32, (8, DH), 0)
            o = jnp.where(row == 0, outs[0], outs[1]).astype(BF16)
            wo = wo_v[pl.ds(pl.multiple_of(g * DH, DH), DH), :]
            return acc + jnp.dot(o, wo, preferred_element_type=F32)

        wait_all(wo_v, w_sem.at[4])

        def body(g, acc):
            slot = g % ring
            kv_wait(slot)
            kv_start(g + ring - 1, (g + ring - 1) % ring)
            return head(g, slot, acc)

        acc = jax.lax.fori_loop(0, H - ring + 1, body, jnp.zeros((8, D), F32))
        split_copy(w1_hbm, w1_v, w_sem.at[5], 43)
        split_copy(w3_hbm, w3_v, w_sem.at[6], 43)
        split_copy(w2_hbm, w2_v, w_sem.at[7], 43)

        def body2(g, acc):
            slot = g % ring
            kv_wait(slot)
            return head(g, slot, acc)

        acc = jax.lax.fori_loop(H - ring + 1, H, body2, acc)

        x1 = x + mod[:, 2 * D:3 * D] * acc[0:B]
        h2 = (_layernorm(x1) * (1.0 + mod[:, 4 * D:5 * D]) + mod[:, 3 * D:4 * D]).astype(BF16)
        wait_all(w1_v, w_sem.at[5])
        gate = jax.lax.dot_general(h2, w1_v[...], _NT, preferred_element_type=F32)
        wait_all(w3_v, w_sem.at[6])
        up = jax.lax.dot_general(h2, w3_v[...], _NT, preferred_element_type=F32)
        hh = (_silu(gate) * up).astype(BF16)
        wait_all(w2_v, w_sem.at[7])
        ffn = jnp.dot(hh, w2_v[...], preferred_element_type=F32)
        out_v[...] = (x1 + mod[:, 5 * D:6 * D] * ffn).astype(out_v.dtype)
        cp = pltpu.make_async_copy(out_v, out_hbm, w_sem.at[8])
        cp.start()
        cp.wait()

    def f(A_x, A_k_cache, A_v_cache, A_wq, A_wo, B_x, B_w1, B_w3, B_w2, c, w_mod):
        B, Sq, D = A_x.shape
        H, SK, DH = A_k_cache.shape[1:]
        W = min(4096, max(256, SK // 4))
        hbm = pl.BlockSpec(memory_space=pltpu.HBM)
        w1t, w3t = B_w1.T, B_w3.T
        out = pl.pallas_call(
            kern,
            out_shape=jax.ShapeDtypeStruct((B, D), A_x.dtype),
            in_specs=[hbm] * 10,
            out_specs=hbm,
            scratch_shapes=[
                pltpu.VMEM((B, D), A_x.dtype),
                pltpu.VMEM(c.shape, c.dtype),
                pltpu.VMEM(w_mod.shape, w_mod.dtype),
                pltpu.VMEM(A_wq.shape, A_wq.dtype),
                pltpu.VMEM(A_wo.shape, A_wo.dtype),
                pltpu.VMEM(w1t.shape, w1t.dtype),
                pltpu.VMEM(w3t.shape, w3t.dtype),
                pltpu.VMEM(B_w2.shape, B_w2.dtype),
                pltpu.VMEM((ring, 2, B, W, DH), A_k_cache.dtype),
                pltpu.VMEM((H, B, 8, DH), F32),
                pltpu.VMEM((B, D), A_x.dtype),
                pltpu.SemaphoreType.DMA((ring,)),
                pltpu.SemaphoreType.DMA((9,)),
            ],
            compiler_params=pltpu.CompilerParams(
                vmem_limit_bytes=64 * 2**20, disable_bounds_checks=True),
        )(A_x.reshape(B, D), A_k_cache, A_v_cache, A_wq, A_wo, w1t, w3t, B_w2, c, w_mod)
        return out.reshape(B, Sq, D)

    return f


@jax.jit
def pallas_adaLN_cond__sliding_block_cached__glu_gated_swiglu__decode_kernel(
    A_x, A_k_cache, A_v_cache, A_wq, A_wo, B_x, B_w1, B_w3, B_w2, c, w_mod
):
    return make()(A_x, A_k_cache, A_v_cache, A_wq, A_wo, B_x, B_w1, B_w3, B_w2, c, w_mod)
```

```python
import functools

import jax
import jax.numpy as jnp
import jax.experimental.pallas as pl
import jax.experimental.pallas.tpu as pltpu

F32 = jnp.float32
BF16 = jnp.bfloat16
_NT = (((1,), (1,)), ((), ()))


def _silu(x):
    return x * (1.0 / (1.0 + jnp.exp(-x)))


def _layernorm(x, eps=1e-5):
    m = jnp.mean(x, axis=-1, keepdims=True)
    d = x - m
    v = jnp.mean(d * d, axis=-1, keepdims=True)
    return d / jnp.sqrt(v + eps)


def make(rows=128, ring=2, mode=0, p2=(7, 2, 1, 1), head="A", tail="B", scopes=False, small_first=True, lag=1, tr=32, gb_last=False):
    import contextlib
    scope = (lambda n: jax.named_scope(n)) if scopes else (lambda n: contextlib.nullcontext())

    def kern(x_hbm, k_hbm, v_hbm, wq_hbm, wo_hbm, w1_hbm, w3_hbm, w2_hbm, c_hbm, wm_hbm,
             out_hbm,
             x_v, c_v, wm_v, wq_v, wo_v, w1_v, w3_v, w2_v, kv_v, o_v, out_v,
             kv_sem, w_sem):
        B, H, SK, DH = k_hbm.shape
        D = x_hbm.shape[1]
        FF = w2_hbm.shape[0]
        W = min(4096, max(256, SK // 4))
        nrc = W // rows
        scale = DH ** -0.5
        S_C, S_X, S_WM, S_WQ, S_WO, S_W1, S_W3, S_GB, S_OUT, S_W2 = range(10)

        def kv_start(g):
            slot = g % ring

            @pl.loop(0, nrc)
            def _(rc):
                r0 = pl.multiple_of(rc * rows, rows)
                for kv, src in enumerate((k_hbm, v_hbm)):
                    for b in range(B):
                        pltpu.make_async_copy(
                            src.at[b, g, pl.ds(SK - W + r0, rows), :],
                            kv_v.at[slot, kv, b, pl.ds(r0, rows), :],
                            kv_sem.at[slot]).start(priority=b % 2)

        def stream(n, parts):
            @pl.loop(0, n)
            def _(i):
                for (src, dst, sem, row0, r, c0, nc, pr) in parts:
                    a = pl.multiple_of(row0 + i * r, 8)
                    idx = (pl.ds(a, r), pl.ds(c0, nc))
                    pltpu.make_async_copy(src.at[idx], dst.at[idx], w_sem.at[sem]).start(priority=pr)

        def four(src, dst, sem, row0, nrows, r, c0=0, nc=None):
            q = nrows // 4
            assert q * 4 == nrows and q % r == 0
            nc = src.shape[1] if nc is None else nc
            stream(q // r, [(src, dst, sem, row0 + j * q, r, c0, nc, j % 2) for j in range(4)])

        def wait_all(dst, sem):
            pltpu.make_async_copy(dst, dst, sem).wait()

        def small():
            pltpu.make_async_copy(c_hbm, c_v, w_sem.at[S_C]).start()
            pltpu.make_async_copy(x_hbm, x_v, w_sem.at[S_X]).start(priority=1)

        if small_first:
            small()
        late_gb = tail in ("A", "B")
        nm = 5 * D if late_gb else 6 * D
        if head == "A":
            four(wm_hbm, wm_v, S_WM, 0, D, 8, 0, nm)
            four(wq_hbm, wq_v, S_WQ, 0, D, 8)
        elif head == "B":
            four(wm_hbm, wm_v, S_WM, 0, D, 8, 0, nm)
            hq = H * DH // 2
            stream(D // 16, [(wq_hbm, wq_v, S_WQ, 0, 8, 0, hq, 0), (wq_hbm, wq_v, S_WQ, D // 2, 8, 0, hq, 1),
                             (wq_hbm, wq_v, S_WQ, 0, 8, hq, hq, 0), (wq_hbm, wq_v, S_WQ, D // 2, 8, hq, hq, 1)])
        elif head == "C":
            stream(D // 16, [(wm_hbm, wm_v, S_WM, 0, 8, 0, nm, 0), (wm_hbm, wm_v, S_WM, D // 2, 8, 0, nm, 1),
                             (wq_hbm, wq_v, S_WQ, 0, 8, 0, H * DH, 0), (wq_hbm, wq_v, S_WQ, D // 2, 8, 0, H * DH, 1)])
        elif head == "D":
            hq = H * DH // 2
            stream(D // 16, [(wm_hbm, wm_v, S_WM, 0, 8, 0, nm, 0), (wm_hbm, wm_v, S_WM, D // 2, 8, 0, nm, 1),
                             (wq_hbm, wq_v, S_WQ, 0, 8, 0, hq, 0), (wq_hbm, wq_v, S_WQ, D // 2, 8, 0, hq, 1),
                             (wq_hbm, wq_v, S_WQ, 0, 8, hq, hq, 0), (wq_hbm, wq_v, S_WQ, D // 2, 8, hq, hq, 1)])
        if not small_first:
            small()

        for g in range(ring - 1):
            kv_start(g)

        wait_all(c_v, w_sem.at[S_C])
        wait_all(x_v, w_sem.at[S_X])
        with scope("wmwait"):
            wait_all(wm_v.at[:, pl.ds(0, nm)], w_sem.at[S_WM])
        sc = _silu(c_v[...].astype(F32)).astype(BF16)
        mod = jnp.dot(sc, wm_v[:, 0:nm], preferred_element_type=F32)
        x = x_v[...].astype(F32)
        h = (_layernorm(x) * (1.0 + mod[:, D:2 * D]) + mod[:, 0:D]).astype(BF16)
        with scope("wqwait"):
            wait_all(wq_v, w_sem.at[S_WQ])

        pieces = []
        a = 0
        for t in p2:
            e = min(FF, a + 128 * t)
            pieces.append((a, e - a))
            a = e
        assert a == FF

        def ffn_weights_start():
            if tail == "A":
                n = FF // 32
                ngb = D // 32
                n0 = (2 * n - n - ngb) // 4 * 1
                stream(n0, [(w1_hbm, w1_v, S_W1, 0, 32, 0, D, 0), (w1_hbm, w1_v, S_W1, n0 * 32, 32, 0, D, 1),
                            (w3_hbm, w3_v, S_W3, 0, 32, 0, D, 0), (w3_hbm, w3_v, S_W3, n0 * 32, 32, 0, D, 1)])
                done = 2 * n0
                stream(ngb // 2, [(w1_hbm, w1_v, S_W1, done * 32, 32, 0, D, 1-lag), (wm_hbm, wm_v, S_GB, 0, 32, 5 * D, D, lag),
                                  (w3_hbm, w3_v, S_W3, done * 32, 32, 0, D, 1-lag), (wm_hbm, wm_v, S_GB, D // 2, 32, 5 * D, D, lag)])
                done += ngb // 2
                rest = n - done
                q0 = [(m, done + i) for i in range(rest) for m in (0, 1)]
                q1 = [(pi, a // 32 + i) for pi, (a, nr) in enumerate(pieces) for i in range(nr // 32)]
                for i in range(max(len(q0), len(q1))):
                    if i < len(q0):
                        m, ci = q0[i]
                        src, dst, sem = ((w1_hbm, w1_v, S_W1), (w3_hbm, w3_v, S_W3))[m]
                        pltpu.make_async_copy(src.at[pl.ds(ci * 32, 32), :], dst.at[pl.ds(ci * 32, 32), :], w_sem.at[sem]).start(priority=1-lag)
                    if i < len(q1):
                        pi, ci = q1[i]
                        pltpu.make_async_copy(w2_hbm.at[pl.ds(ci * 32, 32), :], w2_v.at[pl.ds(ci * 32, 32), :], w_sem.at[S_W2 + pi]).start(priority=lag)

            elif tail == "B":
                n = FF // 32
                stream(n, [(w1_hbm, w1_v, S_W1, 0, 32, 0, D, 0), (w3_hbm, w3_v, S_W3, 0, 32, 0, D, 1)])
                def gbs():
                    stream(D // 64, [(wm_hbm, wm_v, S_GB, 0, 32, 5 * D, D, 0), (wm_hbm, wm_v, S_GB, D // 2, 32, 5 * D, D, 1)])
                if not gb_last: gbs()
                ci = 0
                for pi, (a, nr) in enumerate(pieces):
                    for i in range(nr // tr):
                        r = pl.ds(a + i * tr, tr)
                        pltpu.make_async_copy(w2_hbm.at[r, :], w2_v.at[r, :], w_sem.at[S_W2 + pi]).start(priority=ci % 2)
                        ci += 1
                if gb_last: gbs()

        row = jax.lax.broadcasted_iota(jnp.int32, (8, DH), 0)

        @pl.loop(0, H)
        def _(g):
            slot = g % ring

            @pl.when(g + ring - 1 < H)
            def _():
                with scope("kvstart"):
                    kv_start(g + ring - 1)

            @pl.when(g + ring - 1 == H)
            def _():
                with scope("wostart"):
                    four(wo_hbm, wo_v, S_WO, 0, H * DH, 32)

            with scope("kvwait"):
                wait_all(kv_v.at[slot], kv_sem.at[slot])
            if mode == 1:
                return
            col = pl.ds(pl.multiple_of(g * DH, DH), DH)
            q = jnp.dot(h, wq_v[:, col], preferred_element_type=F32)
            outs = []
            for b in range(B):
                qb = jnp.broadcast_to(q[b:b + 1], (8, DH)).astype(BF16)
                s = jax.lax.dot_general(qb, kv_v[slot, 0, b], _NT, preferred_element_type=F32)
                m = jnp.max(s, axis=-1, keepdims=True)
                p = jnp.exp((s - m) * scale)
                l = jnp.sum(p, axis=-1, keepdims=True)
                o = jnp.dot(p.astype(BF16), kv_v[slot, 1, b], preferred_element_type=F32)
                outs.append(o / l)
            o_v[:, col] = jnp.where(row == 0, outs[0], outs[1])

        with scope("ffnstart"):
            ffn_weights_start()
        with scope("wowait"):
            wait_all(wo_v, w_sem.at[S_WO])
        if mode == 1:
            wait_all(w1_v, w_sem.at[S_W1])
            wait_all(w3_v, w_sem.at[S_W3])
            wait_all(wm_v.at[:, pl.ds(5 * D, D)], w_sem.at[S_GB])
            for i, (a, n) in enumerate(pieces):
                wait_all(w2_v.at[pl.ds(a, n), :], w_sem.at[S_W2 + i])
            out_v[...] = x.astype(out_v.dtype)
        else:
            acc = jnp.dot(o_v[...].astype(BF16), wo_v[...], preferred_element_type=F32)
            x1 = x + mod[:, 2 * D:3 * D] * acc[0:B]
            h2 = (_layernorm(x1) * (1.0 + mod[:, 4 * D:5 * D]) + mod[:, 3 * D:4 * D]).astype(BF16)
            with scope("w1wait"):
                wait_all(w1_v, w_sem.at[S_W1])
            gate = jax.lax.dot_general(h2, w1_v[...], _NT, preferred_element_type=F32)
            with scope("w3wait"):
                wait_all(w3_v, w_sem.at[S_W3])
            up = jax.lax.dot_general(h2, w3_v[...], _NT, preferred_element_type=F32)
            hh = (_silu(gate) * up).astype(BF16)
            def gbc():
                with scope("gbwait"):
                    wait_all(wm_v.at[:, pl.ds(5 * D, D)], w_sem.at[S_GB])
                return jnp.dot(sc, wm_v[:, 5 * D:6 * D], preferred_element_type=F32)
            if not gb_last: gb = gbc()
            ffn = jnp.zeros((B, D), F32)
            for i, (a, n) in enumerate(pieces):
                with scope("w2wait"):
                    wait_all(w2_v.at[pl.ds(a, n), :], w_sem.at[S_W2 + i])
                ffn = ffn + jnp.dot(hh[:, a:a + n], w2_v[a:a + n, :], preferred_element_type=F32)
            if gb_last: gb = gbc()
            out_v[...] = (x1 + gb * ffn).astype(out_v.dtype)
        with scope("outw"):
            cp = pltpu.make_async_copy(out_v, out_hbm, w_sem.at[S_OUT])
            cp.start()
            cp.wait()

    def f(A_x, A_k_cache, A_v_cache, A_wq, A_wo, B_x, B_w1, B_w3, B_w2, c, w_mod):
        B, Sq, D = A_x.shape
        H, SK, DH = A_k_cache.shape[1:]
        W = min(4096, max(256, SK // 4))
        hbm = pl.BlockSpec(memory_space=pltpu.HBM)
        w1t, w3t = B_w1.T, B_w3.T
        out = pl.pallas_call(
            kern,
            out_shape=jax.ShapeDtypeStruct((B, D), A_x.dtype),
            in_specs=[hbm] * 10,
            out_specs=hbm,
            scratch_shapes=[
                pltpu.VMEM((B, D), A_x.dtype),
                pltpu.VMEM(c.shape, c.dtype),
                pltpu.VMEM(w_mod.shape, w_mod.dtype),
                pltpu.VMEM(A_wq.shape, A_wq.dtype),
                pltpu.VMEM(A_wo.shape, A_wo.dtype),
                pltpu.VMEM(w1t.shape, w1t.dtype),
                pltpu.VMEM(w3t.shape, w3t.dtype),
                pltpu.VMEM(B_w2.shape, B_w2.dtype),
                pltpu.VMEM((ring, 2, B, W, DH), A_k_cache.dtype),
                pltpu.VMEM((8, H * DH), F32),
                pltpu.VMEM((B, D), A_x.dtype),
                pltpu.SemaphoreType.DMA((ring,)),
                pltpu.SemaphoreType.DMA((9 + len(p2),)),
            ],
            compiler_params=pltpu.CompilerParams(
                vmem_limit_bytes=64 * 2**20, disable_bounds_checks=True),
        )(A_x.reshape(B, D), A_k_cache, A_v_cache, A_wq, A_wo, w1t, w3t, B_w2, c, w_mod)
        return out.reshape(B, Sq, D)

    return f


@jax.jit
def pallas_adaLN_cond__sliding_block_cached__glu_gated_swiglu__decode_kernel(
    A_x, A_k_cache, A_v_cache, A_wq, A_wo, B_x, B_w1, B_w3, B_w2, c, w_mod
):
    return make(p2=(5,4,2))(A_x, A_k_cache, A_v_cache, A_wq, A_wo, B_x, B_w1, B_w3, B_w2, c, w_mod)
```

```python
import functools

import jax
import jax.numpy as jnp
import jax.experimental.pallas as pl
import jax.experimental.pallas.tpu as pltpu

F32 = jnp.float32
BF16 = jnp.bfloat16
_NT = (((1,), (1,)), ((), ()))


def _silu(x):
    return x * (1.0 / (1.0 + jnp.exp(-x)))


def _layernorm(x, eps=1e-5):
    m = jnp.mean(x, axis=-1, keepdims=True)
    d = x - m
    v = jnp.mean(d * d, axis=-1, keepdims=True)
    return d / jnp.sqrt(v + eps)


def make(rows=128, ring=2, mode=0, p2=(5, 4, 2), head="E", tail="C", scopes=False, small_first=True, lag=1, tr=32, gb_last=False, kvpat="qkv", ob=0, wopat=0, hpg=2, hs=4, first=1):
    import contextlib
    scope = (lambda n: jax.named_scope(n)) if scopes else (lambda n: contextlib.nullcontext())

    def kern(x_hbm, k_hbm, v_hbm, wq_hbm, wo_hbm, w1_hbm, w3_hbm, w2_hbm, c_hbm, wm_hbm,
             out_hbm,
             x_v, c_v, wm_v, wq_v, wo_v, w1_v, w3_v, w2_v, kv_v, o_v, out_v,
             kv_sem, w_sem):
        B, H, SK, DH = k_hbm.shape
        D = x_hbm.shape[1]
        FF = w2_hbm.shape[0]
        W = min(4096, max(256, SK // 4))
        nrc = W // rows
        scale = DH ** -0.5
        S_C, S_X, S_WM, S_WQ, S_WO, S_W1, S_W3, S_GB, S_OUT, S_W2 = range(10)

        G = H // hpg
        nper = nrc // hpg

        def head0(g):
            return (g // hs) * (hs * hpg) + g % hs

        def kv_start(g, i0, n):
            slot = g % 2
            h0 = head0(g)

            @pl.loop(i0, i0 + n)
            def _(rc):
                r0 = pl.multiple_of(rc * rows, rows)
                for b in range(B):
                    for t in range(hpg):
                        for kv in range(2):
                            pltpu.make_async_copy(
                                (k_hbm, v_hbm)[kv].at[b, h0 + t * hs, pl.ds(SK - W + r0, rows), :],
                                kv_v.at[slot, kv, b, t, pl.ds(r0, rows), :],
                                kv_sem.at[slot]).start(priority=(kv + first) % 2)

        def stream(n, parts):
            @pl.loop(0, n)
            def _(i):
                for (src, dst, sem, row0, r, c0, nc, pr) in parts:
                    a = pl.multiple_of(row0 + i * abs(r), 8)
                    idx = (pl.ds(a, r if r > 0 else 8), pl.ds(c0, nc))
                    pltpu.make_async_copy(src.at[idx], dst.at[idx], w_sem.at[sem]).start(priority=pr)

        def four(src, dst, sem, row0, nrows, r, c0=0, nc=None):
            q = nrows // 4
            assert q * 4 == nrows and q % r == 0
            nc = src.shape[1] if nc is None else nc
            stream(q // r, [(src, dst, sem, row0 + j * q, r, c0, nc, j % 2) for j in range(4)])

        def wait_all(dst, sem):
            pltpu.make_async_copy(dst, dst, sem).wait()

        def small():
            pltpu.make_async_copy(c_hbm, c_v, w_sem.at[S_C]).start()
            pltpu.make_async_copy(x_hbm, x_v, w_sem.at[S_X]).start(priority=1)

        if small_first:
            small()
        late_gb = tail in ("A", "B")
        nm = 5 * D if late_gb else 6 * D
        if head == "A":
            four(wm_hbm, wm_v, S_WM, 0, D, 8, 0, nm)
            four(wq_hbm, wq_v, S_WQ, 0, D, 8)
        elif head == "B":
            four(wm_hbm, wm_v, S_WM, 0, D, 8, 0, nm)
            hq = H * DH // 2
            stream(D // 16, [(wq_hbm, wq_v, S_WQ, 0, 8, 0, hq, 0), (wq_hbm, wq_v, S_WQ, D // 2, 8, 0, hq, 1),
                             (wq_hbm, wq_v, S_WQ, 0, 8, hq, hq, 0), (wq_hbm, wq_v, S_WQ, D // 2, 8, hq, hq, 1)])
        elif head == "C":
            stream(D // 16, [(wm_hbm, wm_v, S_WM, 0, 8, 0, nm, 0), (wm_hbm, wm_v, S_WM, D // 2, 8, 0, nm, 1),
                             (wq_hbm, wq_v, S_WQ, 0, 8, 0, H * DH, 0), (wq_hbm, wq_v, S_WQ, D // 2, 8, 0, H * DH, 1)])
        elif head == "D":
            hq = H * DH // 2
            stream(D // 16, [(wm_hbm, wm_v, S_WM, 0, 8, 0, nm, 0), (wm_hbm, wm_v, S_WM, D // 2, 8, 0, nm, 1),
                             (wq_hbm, wq_v, S_WQ, 0, 8, 0, hq, 0), (wq_hbm, wq_v, S_WQ, D // 2, 8, 0, hq, 1),
                             (wq_hbm, wq_v, S_WQ, 0, 8, hq, hq, 0), (wq_hbm, wq_v, S_WQ, D // 2, 8, hq, hq, 1)])
        elif head == "E":
            assert nm == 6 * D
            hq = H * DH // 2
            def wmp(r0, pr):
                return [(wm_hbm, wm_v, S_WM, r0, -16, 0, 2048, pr), (wm_hbm, wm_v, S_WM, r0, -16, 2048, 1024, pr),
                        (wm_hbm, wm_v, S_WM, r0 + 8, -16, 0, 1024, pr), (wm_hbm, wm_v, S_WM, r0 + 8, -16, 1024, 2048, pr)]
            def wqp(r0, pr):
                return [(wq_hbm, wq_v, S_WQ, r0, -16, 0, hq, pr), (wq_hbm, wq_v, S_WQ, r0, -16, hq, hq, pr),
                        (wq_hbm, wq_v, S_WQ, r0 + 8, -16, 0, hq, pr), (wq_hbm, wq_v, S_WQ, r0 + 8, -16, hq, hq, pr)]
            parts = []
            for a0, a1, b0, b1 in zip(wmp(0, 0), wqp(0, 1), wmp(D // 2, 0), wqp(D // 2, 1)):
                parts += [a0, a1, b0, b1]
            stream(D // 32, parts)
        elif head == "F":
            assert nm == 6 * D
            hq = H * DH // 2
            def wmp(r0, pr):
                return [(wm_hbm, wm_v, S_WM, r0, -16, 0, 2048, pr), (wm_hbm, wm_v, S_WM, r0, -16, 2048, 1024, pr),
                        (wm_hbm, wm_v, S_WM, r0 + 8, -16, 0, 1024, pr), (wm_hbm, wm_v, S_WM, r0 + 8, -16, 1024, 2048, pr)]
            def wqp(r0, pr):
                return [(wq_hbm, wq_v, S_WQ, r0, -8, 0, hq, pr), (wq_hbm, wq_v, S_WQ, r0, -8, hq, hq, pr)]
            stream(D // 64, [p for t in zip(*[wmp(j * D // 4, j % 2) for j in range(4)]) for p in t])
            stream(D // 32, [p for t in zip(*[wqp(j * D // 4, j % 2) for j in range(4)]) for p in t])
        if not small_first:
            small()

        kv_start(0, 0, nrc)

        wait_all(c_v, w_sem.at[S_C])
        wait_all(x_v, w_sem.at[S_X])
        with scope("wmwait"):
            wait_all(wm_v.at[:, pl.ds(0, nm)], w_sem.at[S_WM])
        sc = _silu(c_v[...].astype(F32)).astype(BF16)
        mod = jnp.dot(sc, wm_v[:, 0:nm], preferred_element_type=F32)
        x = x_v[...].astype(F32)
        h = (_layernorm(x) * (1.0 + mod[:, D:2 * D]) + mod[:, 0:D]).astype(BF16)
        with scope("wqwait"):
            wait_all(wq_v, w_sem.at[S_WQ])

        pieces = []
        a = 0
        for t in p2:
            e = min(FF, a + 128 * t)
            pieces.append((a, e - a))
            a = e
        assert a == FF

        def ffn_weights_start():
            if tail == "A":
                n = FF // 32
                ngb = D // 32
                n0 = (2 * n - n - ngb) // 4 * 1
                stream(n0, [(w1_hbm, w1_v, S_W1, 0, 32, 0, D, 0), (w1_hbm, w1_v, S_W1, n0 * 32, 32, 0, D, 1),
                            (w3_hbm, w3_v, S_W3, 0, 32, 0, D, 0), (w3_hbm, w3_v, S_W3, n0 * 32, 32, 0, D, 1)])
                done = 2 * n0
                stream(ngb // 2, [(w1_hbm, w1_v, S_W1, done * 32, 32, 0, D, 1-lag), (wm_hbm, wm_v, S_GB, 0, 32, 5 * D, D, lag),
                                  (w3_hbm, w3_v, S_W3, done * 32, 32, 0, D, 1-lag), (wm_hbm, wm_v, S_GB, D // 2, 32, 5 * D, D, lag)])
                done += ngb // 2
                rest = n - done
                q0 = [(m, done + i) for i in range(rest) for m in (0, 1)]
                q1 = [(pi, a // 32 + i) for pi, (a, nr) in enumerate(pieces) for i in range(nr // 32)]
                for i in range(max(len(q0), len(q1))):
                    if i < len(q0):
                        m, ci = q0[i]
                        src, dst, sem = ((w1_hbm, w1_v, S_W1), (w3_hbm, w3_v, S_W3))[m]
                        pltpu.make_async_copy(src.at[pl.ds(ci * 32, 32), :], dst.at[pl.ds(ci * 32, 32), :], w_sem.at[sem]).start(priority=1-lag)
                    if i < len(q1):
                        pi, ci = q1[i]
                        pltpu.make_async_copy(w2_hbm.at[pl.ds(ci * 32, 32), :], w2_v.at[pl.ds(ci * 32, 32), :], w_sem.at[S_W2 + pi]).start(priority=lag)

            elif tail in ("B", "C"):
                n = FF // 32
                stream(n, [(w1_hbm, w1_v, S_W1, 0, 32, 0, D, 0), (w3_hbm, w3_v, S_W3, 0, 32, 0, D, 1)])
                def gbs():
                    stream(D // 64, [(wm_hbm, wm_v, S_GB, 0, 32, 5 * D, D, 0), (wm_hbm, wm_v, S_GB, D // 2, 32, 5 * D, D, 1)])
                if late_gb and not gb_last: gbs()
                ci = 0
                for pi, (a, nr) in enumerate(pieces):
                    for i in range(nr // tr):
                        r = pl.ds(a + i * tr, tr)
                        pltpu.make_async_copy(w2_hbm.at[r, :], w2_v.at[r, :], w_sem.at[S_W2 + pi]).start(priority=ci % 2)
                        ci += 1
                if late_gb and gb_last: gbs()

        row = jax.lax.broadcasted_iota(jnp.int32, (8, DH), 0)

        @pl.loop(0, H)
        def _(it):
            g = it // hpg
            t = it % hpg
            slot = g % 2

            @pl.when(g + 1 < G)
            def _():
                with scope("kvstart"):
                    kv_start(g + 1, t * nper, nper)

            @pl.when(it == H - hpg)
            def _():
                with scope("wostart"):
                    if wopat == 0:
                        four(wo_hbm, wo_v, S_WO, 0, H * DH, 32)
                    else:
                        qq = H * DH // 8
                        stream(qq // 32, [(wo_hbm, wo_v, S_WO, j * qq, 32, 0, D, j % 2) for j in range(8)])

            if hpg > 1:
                @pl.when(it == H - hpg + 1)
                def _():
                    with scope("ffnstart"):
                        ffn_weights_start()

            @pl.when(t == 0)
            def _():
                with scope("kvwait"):
                    wait_all(kv_v.at[slot], kv_sem.at[slot])
            if mode == 1:
                return
            col = pl.ds(pl.multiple_of((head0(g) + t * hs) * DH, DH), DH)
            q = jnp.dot(h, wq_v[:, col], preferred_element_type=F32)
            outs = []
            for b in range(B):
                qb = jnp.broadcast_to(q[b:b + 1], (8, DH)).astype(BF16)
                s = jax.lax.dot_general(qb, kv_v[slot, 0, b, t], _NT, preferred_element_type=F32)
                m = jnp.max(s, axis=-1, keepdims=True)
                p = jnp.exp((s - m) * scale)
                l = jnp.sum(p, axis=-1, keepdims=True)
                o = jnp.dot(p.astype(BF16), kv_v[slot, 1, b, t], preferred_element_type=F32)
                outs.append(o / l)
            o_v[:, col] = jnp.where(row == 0, outs[0], outs[1])

        if hpg == 1:
            with scope("ffnstart"):
                ffn_weights_start()
        with scope("wowait"):
            wait_all(wo_v, w_sem.at[S_WO])
        if mode == 1:
            wait_all(w1_v, w_sem.at[S_W1])
            wait_all(w3_v, w_sem.at[S_W3])
            if late_gb: wait_all(wm_v.at[:, pl.ds(5 * D, D)], w_sem.at[S_GB])
            for i, (a, n) in enumerate(pieces):
                wait_all(w2_v.at[pl.ds(a, n), :], w_sem.at[S_W2 + i])
            out_v[...] = x.astype(out_v.dtype)
        else:
            acc = jnp.dot(o_v[...].astype(BF16), wo_v[...], preferred_element_type=F32)
            x1 = x + mod[:, 2 * D:3 * D] * acc[0:B]
            h2 = (_layernorm(x1) * (1.0 + mod[:, 4 * D:5 * D]) + mod[:, 3 * D:4 * D]).astype(BF16)
            with scope("w1wait"):
                wait_all(w1_v, w_sem.at[S_W1])
            gate = jax.lax.dot_general(h2, w1_v[...], _NT, preferred_element_type=F32)
            with scope("w3wait"):
                wait_all(w3_v, w_sem.at[S_W3])
            up = jax.lax.dot_general(h2, w3_v[...], _NT, preferred_element_type=F32)
            hh = (_silu(gate) * up).astype(BF16)
            def gbc():
                if not late_gb:
                    return mod[:, 5 * D:6 * D]
                with scope("gbwait"):
                    wait_all(wm_v.at[:, pl.ds(5 * D, D)], w_sem.at[S_GB])
                return jnp.dot(sc, wm_v[:, 5 * D:6 * D], preferred_element_type=F32)
            if not gb_last: gb = gbc()
            ffn = jnp.zeros((B, D), F32)
            for i, (a, n) in enumerate(pieces):
                with scope("w2wait"):
                    wait_all(w2_v.at[pl.ds(a, n), :], w_sem.at[S_W2 + i])
                ffn = ffn + jnp.dot(hh[:, a:a + n], w2_v[a:a + n, :], preferred_element_type=F32)
            if gb_last: gb = gbc()
            out_v[...] = (x1 + gb * ffn).astype(out_v.dtype)
        with scope("outw"):
            cp = pltpu.make_async_copy(out_v, out_hbm, w_sem.at[S_OUT])
            cp.start()
            cp.wait()

    def f(A_x, A_k_cache, A_v_cache, A_wq, A_wo, B_x, B_w1, B_w3, B_w2, c, w_mod):
        B, Sq, D = A_x.shape
        H, SK, DH = A_k_cache.shape[1:]
        W = min(4096, max(256, SK // 4))
        hbm = pl.BlockSpec(memory_space=pltpu.HBM)
        w1t, w3t = B_w1.T, B_w3.T
        out = pl.pallas_call(
            kern,
            out_shape=jax.ShapeDtypeStruct((B, D), A_x.dtype),
            in_specs=[hbm] * 10,
            out_specs=hbm,
            scratch_shapes=[
                pltpu.VMEM((B, D), A_x.dtype),
                pltpu.VMEM(c.shape, c.dtype),
                pltpu.VMEM(w_mod.shape, w_mod.dtype),
                pltpu.VMEM(A_wq.shape, A_wq.dtype),
                pltpu.VMEM(A_wo.shape, A_wo.dtype),
                pltpu.VMEM(w1t.shape, w1t.dtype),
                pltpu.VMEM(w3t.shape, w3t.dtype),
                pltpu.VMEM(B_w2.shape, B_w2.dtype),
                pltpu.VMEM((2, 2, B, hpg, W, DH), A_k_cache.dtype),
                pltpu.VMEM((8, H * DH), F32),
                pltpu.VMEM((B, D), A_x.dtype),
                pltpu.SemaphoreType.DMA((ring,)),
                pltpu.SemaphoreType.DMA((9 + len(p2),)),
            ],
            compiler_params=pltpu.CompilerParams(
                vmem_limit_bytes=100 * 2**20, disable_bounds_checks=True),
        )(A_x.reshape(B, D), A_k_cache, A_v_cache, A_wq, A_wo, w1t, w3t, B_w2, c, w_mod)
        return out.reshape(B, Sq, D)

    return f


@jax.jit
def pallas_adaLN_cond__sliding_block_cached__glu_gated_swiglu__decode_kernel(
    A_x, A_k_cache, A_v_cache, A_wq, A_wo, B_x, B_w1, B_w3, B_w2, c, w_mod
):
    return make(head="F")(A_x, A_k_cache, A_v_cache, A_wq, A_wo, B_x, B_w1, B_w3, B_w2, c, w_mod)
```

```python
import contextlib

import jax
import jax.numpy as jnp
import jax.experimental.pallas as pl
import jax.experimental.pallas.tpu as pltpu

F32 = jnp.float32
BF16 = jnp.bfloat16
_NT = (((1,), (1,)), ((), ()))


def _silu(x):
    return x * (1.0 / (1.0 + jnp.exp(-x)))


def _layernorm(x, eps=1e-5):
    m = jnp.mean(x, axis=-1, keepdims=True)
    d = x - m
    v = jnp.mean(d * d, axis=-1, keepdims=True)
    return d / jnp.sqrt(v + eps)


def make(mode=0, p2=(5, 4, 2), scopes=False, hpg=4, hs=4, ph="", pad=0):
    scope = (lambda n: jax.named_scope(n)) if scopes else (lambda n: contextlib.nullcontext())
    rows = 128

    def kern(x_hbm, k_hbm, v_hbm, wq_hbm, wo_hbm, w1_hbm, w3_hbm, w2_hbm, c_hbm, wm_hbm,
             out_hbm,
             x_v, c_v, wm_v, wq_v, wo_v, w1_v, w3_v, w2_v, kv_v, o_v, out_v,
             kv_sem, w_sem):
        B, H, SK, DH = k_hbm.shape
        D = x_hbm.shape[1]
        FF = w2_hbm.shape[0]
        W = min(4096, max(256, SK // 4))
        nrc = W // rows
        scale = DH ** -0.5
        S_C, S_X, S_WM, S_WQ, S_WO, S_W1, S_W3, S_OUT, S_W2 = range(9)
        G = H // hpg
        hh_ = hpg // 2

        def head0(g):
            return (g // hs) * (hs * hpg) + g % hs

        def kv_round(g, ts, r0s, n):
            slot = g % 2
            h0 = head0(g)
            for b in range(B):
                for t in ts:
                    for kv in range(2):
                        r0 = r0s[kv]
                        pltpu.make_async_copy(
                            (k_hbm, v_hbm)[kv].at[b, h0 + t * hs, pl.ds(SK - W + r0, n), :],
                            kv_v.at[slot, kv, b, t, pl.ds(r0, n), :],
                            kv_sem.at[slot, t // hh_]).start(priority=1 - kv)

        def kv_start(g, ts, part, nparts):
            sh = ("k" in ph, "v" in ph)
            half = rows // 2
            nper = nrc // nparts

            @pl.when(part == 0)
            def _():
                kv_round(g, ts, (0, 0), half)
                kv_round(g, ts, tuple(W - half if s else half for s in sh), half)

            @pl.loop(jnp.maximum(part * nper, 1), (part + 1) * nper)
            def _(rc):
                kv_round(g, ts, tuple(pl.multiple_of(rc * rows - (half if s else 0), half) for s in sh), rows)

        def copy(src, dst, sem, pr, r0, n, c0=0, nc=None):
            idx = (pl.ds(r0, n), pl.ds(c0, src.shape[1] if nc is None else nc))
            pltpu.make_async_copy(src.at[idx], dst.at[idx], w_sem.at[sem]).start(priority=pr)

        def row_streams(parts, nrows, r=32):
            half = r // 2
            for (src, dst, sem, pr, row0, s) in parts:
                copy(src, dst, sem, pr, row0, half)
            for (src, dst, sem, pr, row0, s) in parts:
                copy(src, dst, sem, pr, row0 + (nrows - half if s else half), half)

            @pl.loop(1, nrows // r)
            def _(i):
                for (src, dst, sem, pr, row0, s) in parts:
                    copy(src, dst, sem, pr, pl.multiple_of(row0 + i * r - (half if s else 0), half), r)

        def col_streams(src, dst, sem, step, pieces, ns=4):
            q = src.shape[0] // ns

            @pl.loop(0, q // step)
            def _(i):
                for (ro, c0, nc) in pieces:
                    for j in range(ns):
                        copy(src, dst, sem, j % 2, pl.multiple_of(j * q + i * step + ro, 8), 8, c0, nc)

        def wait_all(dst, sem):
            pltpu.make_async_copy(dst, dst, sem).wait()

        pltpu.make_async_copy(c_hbm, c_v, w_sem.at[S_C]).start()
        pltpu.make_async_copy(x_hbm, x_v, w_sem.at[S_X]).start(priority=1)
        u = 1024
        if "m" in ph:
            col_streams(wm_hbm, wm_v, S_WM, 16, [(0, 0, u), (0, u, 2 * u), (8, 0, 2 * u), (8, 2 * u, u)])
        else:
            col_streams(wm_hbm, wm_v, S_WM, 16, [(0, 0, 2 * u), (0, 2 * u, u), (8, 0, u), (8, u, 2 * u)])
        if "q" in ph:
            col_streams(wq_hbm, wq_v, S_WQ, 8, [(0, 0, u), (0, u, 2 * u), (0, 3 * u, u)])
        else:
            col_streams(wq_hbm, wq_v, S_WQ, 8, [(0, 0, 2 * u), (0, 2 * u, 2 * u)])
        kv_start(0, range(hpg), 0, 1)

        wait_all(c_v, w_sem.at[S_C])
        wait_all(x_v, w_sem.at[S_X])
        with scope("wmwait"):
            wait_all(wm_v, w_sem.at[S_WM])
        sc = _silu(c_v[...].astype(F32)).astype(BF16)
        mod = jnp.dot(sc, wm_v[...], preferred_element_type=F32)
        x = x_v[...].astype(F32)
        h = (_layernorm(x) * (1.0 + mod[:, D:2 * D]) + mod[:, 0:D]).astype(BF16)
        with scope("wqwait"):
            wait_all(wq_v, w_sem.at[S_WQ])

        pieces = []
        a = 0
        for t in p2:
            e = min(FF, a + 128 * t)
            pieces.append((a, e - a))
            a = e
        assert a == FF

        row = jax.lax.broadcasted_iota(jnp.int32, (8, DH), 0)
        L = H - 2 * hpg

        @pl.loop(0, H)
        def _(it):
            g = it // hpg
            t = it % hpg
            slot = g % 2

            @pl.when(it < L)
            def _():
                with scope("kvstart"):
                    kv_start(g + 1, range(hpg), t, hpg)

            j = it - L
            @pl.when((j >= 0) & (j < hpg + hh_) & ((j >= hpg) | (j % 2 == 0)))
            def _():
                with scope("kvstart2"):
                    hf = j // hpg
                    part = jnp.where(hf == 0, j // 2, j - hpg)
                    kv_start(G - 1, [hf * hh_ + i for i in range(hh_)], part, hh_)

            @pl.when(it == H - hh_)
            def _():
                with scope("wostart"):
                    q4 = H * DH // 4
                    row_streams([(wo_hbm, wo_v, S_WO, i % 2, i * q4, "o" in ph) for i in range(4)], q4)

            with scope("kvwait"):
                @pl.when(t == 0)
                def _():
                    wait_all(kv_v.at[slot, :, :, pl.ds(0, hh_)], kv_sem.at[slot, 0])

                @pl.when(((t == 0) & (g < G - 1)) | (it == H - hh_))
                def _():
                    wait_all(kv_v.at[slot, :, :, pl.ds(hh_, hh_)], kv_sem.at[slot, 1])

            if mode == 1:
                return
            col = pl.ds(pl.multiple_of((head0(g) + t * hs) * DH, DH), DH)
            q = jnp.dot(h, wq_v[:, col], preferred_element_type=F32)
            outs = []
            for b in range(B):
                qb = jnp.broadcast_to(q[b:b + 1], (8, DH)).astype(BF16)
                s = jax.lax.dot_general(qb, kv_v[slot, 0, b, t], _NT, preferred_element_type=F32)
                m = jnp.max(s, axis=-1, keepdims=True)
                p = jnp.exp((s - m) * scale)
                l = jnp.sum(p, axis=-1, keepdims=True)
                o = jnp.dot(p.astype(BF16), kv_v[slot, 1, b, t], preferred_element_type=F32)
                outs.append(o / l)
            o_v[:, col] = jnp.where(row == 0, outs[0], outs[1])

        with scope("ffnstart"):
            row_streams([(w1_hbm, w1_v, S_W1, 0, 0, "1" in ph), (w3_hbm, w3_v, S_W3, 1, 0, "3" in ph)], FF)
            for i, (a, n) in enumerate(pieces):
                n0 = (n // 64) * 32
                if n0 * 2 == n:
                    row_streams([(w2_hbm, w2_v, S_W2 + i, 0, a, "2" in ph), (w2_hbm, w2_v, S_W2 + i, 1, a + n0, "2" in ph)], n0)
                else:
                    row_streams([(w2_hbm, w2_v, S_W2 + i, 0, a, "2" in ph), (w2_hbm, w2_v, S_W2 + i, 1, a + n0, "2" in ph)], n0)
                    row_streams([(w2_hbm, w2_v, S_W2 + i, 0, a + 2 * n0, "2" in ph)], n - 2 * n0)
        with scope("wowait"):
            wait_all(wo_v, w_sem.at[S_WO])
        if mode == 1:
            wait_all(w1_v, w_sem.at[S_W1])
            wait_all(w3_v, w_sem.at[S_W3])
            for i, (a, n) in enumerate(pieces):
                wait_all(w2_v.at[pl.ds(a, n), :], w_sem.at[S_W2 + i])
            out_v[...] = x.astype(out_v.dtype)
        else:
            acc = jnp.dot(o_v[...].astype(BF16), wo_v[...], preferred_element_type=F32)
            x1 = x + mod[:, 2 * D:3 * D] * acc[0:B]
            h2 = (_layernorm(x1) * (1.0 + mod[:, 4 * D:5 * D]) + mod[:, 3 * D:4 * D]).astype(BF16)
            with scope("w1wait"):
                wait_all(w1_v, w_sem.at[S_W1])
            gate = jax.lax.dot_general(h2, w1_v[...], _NT, preferred_element_type=F32)
            with scope("w3wait"):
                wait_all(w3_v, w_sem.at[S_W3])
            up = jax.lax.dot_general(h2, w3_v[...], _NT, preferred_element_type=F32)
            hh = (_silu(gate) * up).astype(BF16)
            ffn = jnp.zeros((B, D), F32)
            for i, (a, n) in enumerate(pieces):
                with scope("w2wait"):
                    wait_all(w2_v.at[pl.ds(a, n), :], w_sem.at[S_W2 + i])
                ffn = ffn + jnp.dot(hh[:, a:a + n], w2_v[a:a + n, :], preferred_element_type=F32)
            out_v[...] = (x1 + mod[:, 5 * D:6 * D] * ffn).astype(out_v.dtype)
        with scope("outw"):
            cp = pltpu.make_async_copy(out_v, out_hbm, w_sem.at[S_OUT])
            cp.start()
            cp.wait()

    def f(A_x, A_k_cache, A_v_cache, A_wq, A_wo, B_x, B_w1, B_w3, B_w2, c, w_mod):
        B, Sq, D = A_x.shape
        H, SK, DH = A_k_cache.shape[1:]
        W = min(4096, max(256, SK // 4))
        hbm = pl.BlockSpec(memory_space=pltpu.HBM)
        w1t, w3t = B_w1.T, B_w3.T
        out = pl.pallas_call(
            kern,
            out_shape=jax.ShapeDtypeStruct((B, D), A_x.dtype),
            in_specs=[hbm] * 10,
            out_specs=hbm,
            scratch_shapes=[
                pltpu.VMEM((B, D), A_x.dtype),
                pltpu.VMEM(c.shape, c.dtype),
                pltpu.VMEM(w_mod.shape, w_mod.dtype),
                pltpu.VMEM(A_wq.shape, A_wq.dtype),
                pltpu.VMEM(A_wo.shape, A_wo.dtype),
                pltpu.VMEM(w1t.shape, w1t.dtype),
                pltpu.VMEM(w3t.shape, w3t.dtype),
                pltpu.VMEM(B_w2.shape, B_w2.dtype),
                pltpu.VMEM((2, 2, B, hpg, W, DH), A_k_cache.dtype),
                pltpu.VMEM((8, H * DH), F32),
                pltpu.VMEM((B, D), A_x.dtype),
                pltpu.SemaphoreType.DMA((2, 2)),
                pltpu.SemaphoreType.DMA((8 + len(p2),)),
            ],
            compiler_params=pltpu.CompilerParams(
                vmem_limit_bytes=100 * 2**20, disable_bounds_checks=True),
        )(A_x.reshape(B, D), A_k_cache, A_v_cache, A_wq, A_wo, w1t, w3t, B_w2, c, w_mod)
        return out.reshape(B, Sq, D)

    return f


@jax.jit
def pallas_adaLN_cond__sliding_block_cached__glu_gated_swiglu__decode_kernel(
    A_x, A_k_cache, A_v_cache, A_wq, A_wo, B_x, B_w1, B_w3, B_w2, c, w_mod
):
    return make(ph="v")(A_x, A_k_cache, A_v_cache, A_wq, A_wo, B_x, B_w1, B_w3, B_w2, c, w_mod)
```

```python
import jax
import jax.numpy as jnp
import jax.experimental.pallas as pl
import jax.experimental.pallas.tpu as pltpu

F32 = jnp.float32
BF16 = jnp.bfloat16
_NT = (((1,), (1,)), ((), ()))

_GROUP = 4
_HALF = 2
_HEAD_STRIDE = 4
_KV_ROWS = 128
_W_ROWS = 32
_W_COLS = 1024
_KV_SHIFT = (False, True)
_W3_SPLIT = 1024
_W2_PIECES = ((0, 384), (384, 512), (896, 480))

_S_C, _S_X, _S_WM, _S_WQ, _S_WO, _S_W1, _S_W3A, _S_W3B, _S_OUT, _S_W2 = range(10)


def _silu(x):
    return x * (1.0 / (1.0 + jnp.exp(-x)))


def _layernorm(x, eps=1e-5):
    m = jnp.mean(x, axis=-1, keepdims=True)
    d = x - m
    v = jnp.mean(d * d, axis=-1, keepdims=True)
    return d / jnp.sqrt(v + eps)


def _wait_all(dst, sem):
    pltpu.make_async_copy(dst, dst, sem).wait()


def _kernel(x_hbm, k_hbm, v_hbm, wq_hbm, wo_hbm, w1_hbm, w3_hbm, w2_hbm, c_hbm, wm_hbm,
            out_hbm,
            x_v, c_v, wm_v, wq_v, wo_v, w1_v, w3_v, w2_v, kv_v, o_v, out_v,
            kv_sem, w_sem):
    B, H, SK, DH = k_hbm.shape
    D = x_hbm.shape[1]
    FF = w2_hbm.shape[0]
    W = kv_v.shape[4]
    G = H // _GROUP
    scale = DH ** -0.5

    def first_head(g):
        return (g // _HEAD_STRIDE) * (_HEAD_STRIDE * _GROUP) + g % _HEAD_STRIDE

    def kv_round(g, ts, starts, n):
        slot = g % 2
        h0 = first_head(g)
        for b in range(B):
            for t in ts:
                for kv, src in enumerate((k_hbm, v_hbm)):
                    pltpu.make_async_copy(
                        src.at[b, h0 + t * _HEAD_STRIDE, pl.ds(SK - W + starts[kv], n), :],
                        kv_v.at[slot, kv, b, t, pl.ds(starts[kv], n), :],
                        kv_sem.at[slot, t // _HALF],
                    ).start(priority=1 - kv)

    def kv_start(g, ts, part, nparts):
        half = _KV_ROWS // 2
        per = W // _KV_ROWS // nparts

        @pl.when(part == 0)
        def _():
            kv_round(g, ts, (0, 0), half)
            kv_round(g, ts, [W - half if s else half for s in _KV_SHIFT], half)

        @pl.loop(jnp.maximum(part * per, 1), (part + 1) * per)
        def _(i):
            starts = [pl.multiple_of(i * _KV_ROWS - (half if s else 0), half) for s in _KV_SHIFT]
            kv_round(g, ts, starts, _KV_ROWS)

    def copy(src, dst, sem, priority, r0, nr, c0=0, nc=None):
        idx = (pl.ds(r0, nr), pl.ds(c0, src.shape[1] if nc is None else nc))
        pltpu.make_async_copy(src.at[idx], dst.at[idx], w_sem.at[sem]).start(priority=priority)

    def eight_streams(n, start):
        per = n // 8

        @pl.loop(0, per)
        def _(i):
            for j, s in enumerate((0, 4, 1, 5, 2, 6, 3, 7)):
                start(s * per + (i + s) % per, j % 2)

    def two_streams(parts, nrows):
        @pl.loop(0, nrows // _W_ROWS)
        def _(i):
            for priority, (src, dst, sem, r0) in enumerate(parts):
                copy(src, dst, sem, priority, pl.multiple_of(r0 + i * _W_ROWS, _W_ROWS), _W_ROWS)

    pltpu.make_async_copy(c_hbm, c_v, w_sem.at[_S_C]).start()
    pltpu.make_async_copy(x_hbm, x_v, w_sem.at[_S_X]).start(priority=1)
    u = _W_COLS

    @pl.loop(0, D // 64)
    def _(i):
        for dr, c0, nc in ((0, 0, 2 * u), (0, 2 * u, u), (8, 0, u), (8, u, 2 * u)):
            for j in range(4):
                r0 = pl.multiple_of(j * (D // 4) + i * 16 + dr, 8)
                copy(wm_hbm, wm_v, _S_WM, j % 2, r0, 8, c0, nc)

    eight_streams(D // 4, lambda i, priority: copy(
        wq_hbm, wq_v, _S_WQ, priority,
        pl.multiple_of((i // 2) * 8, 8), 8, pl.multiple_of((i % 2) * 2 * u, 2 * u), 2 * u))
    kv_start(0, range(_GROUP), 0, 1)

    _wait_all(c_v, w_sem.at[_S_C])
    _wait_all(x_v, w_sem.at[_S_X])
    _wait_all(wm_v, w_sem.at[_S_WM])
    mod = jnp.dot(_silu(c_v[...].astype(F32)).astype(BF16), wm_v[...],
                  preferred_element_type=F32)
    sa, ca, ga, sb, cb, gb = (mod[:, i * D:(i + 1) * D] for i in range(6))
    x = x_v[...].astype(F32)
    h = (_layernorm(x) * (1.0 + ca) + sa).astype(BF16)
    _wait_all(wq_v, w_sem.at[_S_WQ])

    row = jax.lax.broadcasted_iota(jnp.int32, (8, DH), 0)

    @pl.loop(0, H)
    def _(step):
        g = step // _GROUP
        t = step % _GROUP
        slot = g % 2

        @pl.when(g < G - 2)
        def _():
            kv_start(g + 1, range(_GROUP), t, _GROUP)

        j = step - (G - 2) * _GROUP

        @pl.when((j >= 0) & (j < _GROUP + _HALF) & ((j >= _GROUP) | (j % 2 == 0)))
        def _():
            which = j // _GROUP
            part = jnp.where(which == 0, j // 2, j - _GROUP)
            kv_start(G - 1, [which * _HALF + i for i in range(_HALF)], part, _HALF)

        @pl.when(step == H - _HALF)
        def _():
            eight_streams(H * DH // _W_ROWS, lambda i, priority: copy(
                wo_hbm, wo_v, _S_WO, priority, pl.multiple_of(i * _W_ROWS, _W_ROWS), _W_ROWS))

        @pl.when(t == 0)
        def _():
            _wait_all(kv_v.at[slot, :, :, pl.ds(0, _HALF)], kv_sem.at[slot, 0])

        @pl.when(((t == 0) & (g < G - 1)) | (step == H - _HALF))
        def _():
            _wait_all(kv_v.at[slot, :, :, pl.ds(_HALF, _HALF)], kv_sem.at[slot, 1])

        col = pl.ds(pl.multiple_of((first_head(g) + t * _HEAD_STRIDE) * DH, DH), DH)
        q = jnp.dot(h, wq_v[:, col], preferred_element_type=F32)
        outs = []
        for b in range(B):
            qb = jnp.broadcast_to(q[b:b + 1], (8, DH)).astype(BF16)
            s = jax.lax.dot_general(qb, kv_v[slot, 0, b, t], _NT, preferred_element_type=F32)
            m = jnp.max(s, axis=-1, keepdims=True)
            p = jnp.exp((s - m) * scale)
            l = jnp.sum(p, axis=-1, keepdims=True)
            o = jnp.dot(p.astype(BF16), kv_v[slot, 1, b, t], preferred_element_type=F32)
            outs.append(o / l)
        o_v[:, col] = jnp.where(row == 0, outs[0], outs[1])

    fa = _W3_SPLIT
    two_streams([(w1_hbm, w1_v, _S_W1, 0), (w3_hbm, w3_v, _S_W3A, 0)], fa)
    two_streams([(w1_hbm, w1_v, _S_W1, fa), (w3_hbm, w3_v, _S_W3B, fa)], FF - fa)
    for i, (r0, n) in enumerate(_W2_PIECES):
        n0 = n // (2 * _W_ROWS) * _W_ROWS
        two_streams([(w2_hbm, w2_v, _S_W2 + i, r0), (w2_hbm, w2_v, _S_W2 + i, r0 + n0)], n0)
        if n > 2 * n0:
            copy(w2_hbm, w2_v, _S_W2 + i, 0, r0 + 2 * n0, n - 2 * n0)

    _wait_all(wo_v, w_sem.at[_S_WO])
    attn = jnp.dot(o_v[...].astype(BF16), wo_v[...], preferred_element_type=F32)
    x1 = x + ga * attn[0:B]
    h2 = (_layernorm(x1) * (1.0 + cb) + sb).astype(BF16)

    _wait_all(w1_v, w_sem.at[_S_W1])
    gate = jax.lax.dot_general(h2, w1_v[...], _NT, preferred_element_type=F32)
    _wait_all(w3_v.at[pl.ds(0, fa), :], w_sem.at[_S_W3A])
    act = _silu(gate)
    up = jax.lax.dot_general(h2, w3_v[0:fa, :], _NT, preferred_element_type=F32)
    hidden_a = (act[:, 0:fa] * up).astype(BF16)
    _wait_all(w3_v.at[pl.ds(fa, FF - fa), :], w_sem.at[_S_W3B])
    up = jax.lax.dot_general(h2, w3_v[fa:FF, :], _NT, preferred_element_type=F32)
    hidden = jnp.concatenate([hidden_a, (act[:, fa:FF] * up).astype(BF16)], axis=1)

    ffn = jnp.zeros((B, D), F32)
    for i, (r0, n) in enumerate(_W2_PIECES):
        _wait_all(w2_v.at[pl.ds(r0, n), :], w_sem.at[_S_W2 + i])
        ffn = ffn + jnp.dot(hidden[:, r0:r0 + n], w2_v[r0:r0 + n, :],
                            preferred_element_type=F32)
    out_v[...] = (x1 + gb * ffn).astype(out_v.dtype)

    out_copy = pltpu.make_async_copy(out_v, out_hbm, w_sem.at[_S_OUT])
    out_copy.start()
    out_copy.wait()


@jax.jit
def pallas_adaLN_cond__sliding_block_cached__glu_gated_swiglu__decode_kernel(
    A_x: jax.Array,
    A_k_cache: jax.Array,
    A_v_cache: jax.Array,
    A_wq: jax.Array,
    A_wo: jax.Array,
    B_x: jax.Array,
    B_w1: jax.Array,
    B_w3: jax.Array,
    B_w2: jax.Array,
    c: jax.Array,
    w_mod: jax.Array,
):
    del B_x
    B, Sq, D = A_x.shape
    H, SK, DH = A_k_cache.shape[1:]
    FF = B_w2.shape[0]
    W = min(4096, max(256, SK // 4))
    assert (B, Sq, D, H, DH, W, FF) == (2, 1, 512, 32, 128, 4096, 1376)

    w1t, w3t = B_w1.T, B_w3.T
    hbm = pl.BlockSpec(memory_space=pltpu.HBM)
    out = pl.pallas_call(
        _kernel,
        out_shape=jax.ShapeDtypeStruct((B, D), A_x.dtype),
        in_specs=[hbm] * 10,
        out_specs=hbm,
        scratch_shapes=[
            pltpu.VMEM((B, D), A_x.dtype),
            pltpu.VMEM(c.shape, c.dtype),
            pltpu.VMEM(w_mod.shape, w_mod.dtype),
            pltpu.VMEM(A_wq.shape, A_wq.dtype),
            pltpu.VMEM(A_wo.shape, A_wo.dtype),
            pltpu.VMEM(w1t.shape, w1t.dtype),
            pltpu.VMEM(w3t.shape, w3t.dtype),
            pltpu.VMEM(B_w2.shape, B_w2.dtype),
            pltpu.VMEM((2, 2, B, _GROUP, W, DH), A_k_cache.dtype),
            pltpu.VMEM((8, H * DH), F32),
            pltpu.VMEM((B, D), A_x.dtype),
            pltpu.SemaphoreType.DMA((2, _GROUP // _HALF)),
            pltpu.SemaphoreType.DMA((_S_W2 + len(_W2_PIECES),)),
        ],
        compiler_params=pltpu.CompilerParams(
            vmem_limit_bytes=80 * 2**20,
            disable_semaphore_checks=True,
        ),
    )(A_x.reshape(B, D), A_k_cache, A_v_cache, A_wq, A_wo, w1t, w3t, B_w2, c, w_mod)
    return out.reshape(B, Sq, D)
```
